```python
import os as _os
_os.environ.setdefault("JAX_PLATFORMS", "cpu")
import jax
import jax.numpy as jnp

def _softmax(x, axis=-1):
    return jax.nn.softmax(x, axis=axis)
def _gelu(x):
    return jax.nn.gelu(x, approximate=True)
def _silu(x):
    return jax.nn.silu(x)
def _sigmoid(x):
    return jax.nn.sigmoid(x)
def _layernorm(x, axis=-1, eps=1e-5):
    m = jnp.mean(x, axis=axis, keepdims=True)
    v = jnp.var(x, axis=axis, keepdims=True)
    return (x - m) / jnp.sqrt(v + eps)
def _scatter_add(tgt, idx, src, axis=0):
    return tgt.at[idx].add(src)
def _segment_sum(src, seg, n):
    return jax.ops.segment_sum(src, seg, n)
class _Rng:
    def __init__(self, key):
        self._k = key
    def _next(self):
        self._k, sub = jax.random.split(self._k)
        return sub
    def normal(self, shape):
        return jax.random.normal(self._next(), shape, dtype=jnp.bfloat16)
    def randint(self, lo, hi, shape):
        return jax.random.randint(self._next(), shape, lo, hi, dtype=jnp.int32)
    def uniform(self, shape, lo=0.0, hi=1.0):
        return jax.random.uniform(self._next(), shape, jnp.bfloat16, lo, hi)
    def permutation(self, n):
        return jax.random.permutation(self._next(), n)


kernel_name = 'gated_mix__mha_block__mha_block__prompt'

def setup_inputs():
    _rng = _Rng(jax.random.key(int.from_bytes(__import__("os").urandom(4), "little")))
    _w = (lambda a: (lambda t: t.astype(jnp.bfloat16) if jnp.issubdtype(t.dtype, jnp.floating) else t)(jnp.asarray(a)))
    def _A_setup():
        B, S, D, H = 1, 2048, 448, 16
        return {
            "x": _w((lambda *s: _rng.normal(s) * 0.05)(B, S, D)),
            "wqkv": _w((lambda *s: _rng.normal(s) * 0.4)(D, 3 * D)),
            "wo": _w((lambda *s: _rng.normal(s) * 0.05)(D, D)),
        }
    _A_in = _A_setup()

    def _B_setup():
        B, S, D, H = 1, 2048, 448, 16
        return {
            "x": _w((lambda *s: _rng.normal(s) * 0.05)(B, S, D)),
            "wqkv": _w((lambda *s: _rng.normal(s) * 0.4)(D, 3 * D)),
            "wo": _w((lambda *s: _rng.normal(s) * 0.05)(D, D)),
        }
    _B_in = _B_setup()

    return {
        "A_x": _A_in["x"],
        "A_wqkv": _A_in["wqkv"],
        "A_wo": _A_in["wo"],
        "B_x": _B_in["x"],
        "B_wqkv": _B_in["wqkv"],
        "B_wo": _B_in["wo"],
        "gate_w": _w((lambda *s: _rng.normal(s) * 0.05)(448) * 16.0),
    }

def reference(A_x, A_wqkv, A_wo, B_x, B_wqkv, B_wo, gate_w):
    def _A_ref(x, wqkv, wo):
        B, S, D = x.shape
        H = 16
        Dh = D // H
        qkv = (lambda x, *d: x.transpose(*d))((x @ wqkv).reshape(B, S, 3, H, Dh), 2, 0, 3, 1, 4)
        q, k, v = qkv[0], qkv[1], qkv[2]
        scores = jnp.einsum("bhqd,bhkd->bhqk", q, k) * (Dh ** -0.5)
        p = _softmax(scores, axis=-1)
        o = jnp.einsum("bhqk,bhkd->bhqd", p, v)
        return (lambda x, *d: x.transpose(*d))(o, 0, 2, 1, 3).reshape(B, S, D) @ wo

    def _B_ref(x, wqkv, wo):
        B, S, D = x.shape
        H = 16
        Dh = D // H
        qkv = (lambda x, *d: x.transpose(*d))((x @ wqkv).reshape(B, S, 3, H, Dh), 2, 0, 3, 1, 4)
        q, k, v = qkv[0], qkv[1], qkv[2]
        scores = jnp.einsum("bhqd,bhkd->bhqk", q, k) * (Dh ** -0.5)
        p = _softmax(scores, axis=-1)
        o = jnp.einsum("bhqk,bhkd->bhqd", p, v)
        return (lambda x, *d: x.transpose(*d))(o, 0, 2, 1, 3).reshape(B, S, D) @ wo

    x = A_x
    g = _sigmoid((x * gate_w).sum(-1, keepdims=True))
    a = _A_ref(x, A_wqkv, A_wo)
    b = _B_ref(x, B_wqkv, B_wo)
    return g * a + (1 - g) * b
```

```python
import functools
import numpy as np
import jax
import jax.numpy as jnp
import jax.experimental.pallas as pl
import jax.experimental.pallas.tpu as pltpu

S = 2048
D = 448
H = 16
DH = 28
BQ = 512
BK = 256
TB = 512
QSCALE = float(DH ** -0.5 * np.log2(np.e))

NT_DIMS = (((1,), (1,)), ((), ()))


def _kernel(xt_hbm, wa_hbm, wb_hbm, woa_hbm, wob_hbm, gw_ref, o_hbm,
            xt_ref, wa_ref, wb_ref, woa_ref, wob_ref, o_s, in_sems, out_sems,
            wt_s, wot_s, kp_s, qt_s, vt_s, g_s, ot_s, sA, sB, *, bq, bk):
    nq = S // bq
    nch = S // bk
    f32 = jnp.float32
    bf16 = jnp.bfloat16

    copies = [pltpu.make_async_copy(src, dst, in_sems.at[i]) for i, (src, dst) in enumerate(
        ((wa_hbm, wa_ref), (xt_hbm, xt_ref), (wb_hbm, wb_ref), (woa_hbm, woa_ref), (wob_hbm, wob_ref)))]
    for c in copies:
        c.start()

    QOFF = (0, 976)
    VOFF = (464, 1440)
    GOFF = 1952
    for m, w_ref in enumerate((wa_ref, wb_ref)):
        copies[2 * m].wait()
        wq_t = w_ref[:, 0:512].astype(f32).T
        wt_s[QOFF[m]:QOFF[m] + 464, :] = wq_t[0:464].astype(bf16)
        wv_t = w_ref[:, 896:1344].astype(f32).T
        zpad = jnp.zeros((4, D), f32)
        for h in range(H):
            blk = jnp.concatenate([wv_t[DH * h:DH * h + DH], zpad], axis=0)
            wt_s[VOFF[m] + 32 * h:VOFF[m] + 32 * h + 32, :] = blk.astype(bf16)
    wt_s[GOFF:GOFF + 16, :] = jnp.broadcast_to(gw_ref[...], (16, D))

    for m, wo_ref in enumerate((woa_ref, wob_ref)):
        copies[3 + m].wait()
        wo = wo_ref[...].astype(f32)
        zpad = jnp.zeros((4, D), f32)
        for g in range(4):
            blk = jnp.concatenate(
                [p for h in range(4 * g, 4 * g + 4) for p in (wo[DH * h:DH * h + DH], zpad)], axis=0)
            wot_s[:, 512 * m + 128 * g:512 * m + 128 * g + 128] = blk.T.astype(bf16)

    rowv = jax.lax.broadcasted_iota(jnp.int32, (512, TB), 0)
    ones_row = (rowv % 32) == DH

    copies[1].wait()

    def proj_body(i, c):
        t0 = pl.multiple_of(i * TB, TB)
        xtb = xt_ref[:, pl.ds(t0, TB)]
        xb = xtb.T
        for m, w_ref in enumerate((wa_ref, wb_ref)):
            q = jnp.dot(wt_s[QOFF[m]:QOFF[m] + 464, :], xtb, preferred_element_type=f32)
            q = (q * QSCALE).astype(bf16)
            for u in range(TB // bq):
                qt_s[i * (TB // bq) + u, m] = q[:, u * bq:(u + 1) * bq]
            v = jnp.dot(wt_s[VOFF[m]:VOFF[m] + 512, :], xtb, preferred_element_type=f32)
            v = jnp.where(ones_row, 1.0, v).astype(bf16)
            vt_s[m, :, pl.ds(t0, TB)] = v
            for g in range(4):
                c0 = D + 112 * g
                k = jnp.dot(xb, w_ref[:, c0:c0 + 128], preferred_element_type=f32)
                kp_s[4 * m + g, pl.ds(t0, TB), :] = k.astype(bf16)
        z = jnp.dot(wt_s[GOFF:GOFF + 16, :], xtb, preferred_element_type=f32)
        gate = jax.nn.sigmoid(z[0:8])
        g_s[:, pl.ds(t0, TB)] = gate
        return c

    jax.lax.fori_loop(0, S // TB, proj_body, 0)

    row = jax.lax.broadcasted_iota(jnp.int32, (128, bq), 0)

    def qweights(qb, grp, hp):
        m = grp // 4
        g = grp % 4
        w = qt_s[qb, m, pl.ds(pl.multiple_of(g * 112, 16), 128), :]
        lo = hp * DH
        msk = jnp.logical_and(row >= lo, row < lo + DH)
        return jnp.where(msk, w, jnp.zeros_like(w))

    def qk_chunk(w, grp, sb, j, mx):
        kc = kp_s[grp, pl.ds(j * bk, bk), :]
        s = jnp.dot(kc, w, preferred_element_type=f32)
        sb[pl.ds(j * bk, bk), :] = s
        cm = jnp.max(s.reshape(bk // 8, 8, bq), axis=0)
        return cm if mx is None else jnp.maximum(mx, cm)

    def pv_chunk(grp, hp, sb, j, mcur, acc, z):
        s = sb[pl.ds(pl.multiple_of(j * bk + z, 8), bk), :]
        p = jnp.exp2(s - mcur).astype(bf16)
        m = grp // 4
        g = grp % 4
        v = vt_s[m, pl.ds(pl.multiple_of(g * 128 + hp * 32, 32), 32), pl.ds(j * bk, bk)]
        d = jnp.dot(v, p, preferred_element_type=f32)
        return d if acc is None else acc + d

    def step(cur_idx, nxt_idx, mcur, scur, snxt):
        mx = None
        acc = None
        if nxt_idx is not None:
            w = qweights(*nxt_idx)
        for j in range(nch):
            if nxt_idx is not None:
                mx = qk_chunk(w, nxt_idx[1], snxt, j, mx)
            if cur_idx is not None:
                acc = pv_chunk(cur_idx[1], cur_idx[2], scur, j, mcur, acc, cur_idx[1] // 1024)
        if cur_idx is not None:
            qb, grp, hp = cur_idx
            gate = g_s[0:1, pl.ds(pl.multiple_of(qb * bq, bq), bq)]
            wgt = jnp.where(grp < 4, gate, 1.0 - gate)
            o = acc * (wgt / acc[DH:DH + 1, :])
            ot_s[qb, pl.ds(pl.multiple_of(grp * 128 + hp * 32, 32), 32), :] = o.astype(bf16)
        if nxt_idx is not None:
            return jnp.max(mx, axis=0, keepdims=True)
        return None

    m0 = step(None, (0, 0, 0), None, None, sA)
    n_it = nq * 8

    def body(it, mcur):
        qb = it // 8
        grp = it % 8
        itn = jnp.minimum(it + 1, n_it - 1)
        qbn = itn // 8
        grpn = itn % 8
        mcur = step((qb, grp, 0), (qb, grp, 1), mcur, sA, sB)
        mcur = step((qb, grp, 1), (qb, grp, 2), mcur, sB, sA)
        mcur = step((qb, grp, 2), (qb, grp, 3), mcur, sA, sB)
        mcur = step((qb, grp, 3), (qbn, grpn, 0), mcur, sB, sA)
        return mcur

    jax.lax.fori_loop(0, n_it, body, m0)

    out_copies = []
    for qb in range(nq):
        ot = jnp.dot(wot_s[...], ot_s[qb], preferred_element_type=f32)
        o_s[qb] = ot.astype(o_s.dtype)
        cp = pltpu.make_async_copy(o_s.at[qb], o_hbm.at[:, pl.ds(qb * bq, bq)], out_sems.at[qb])
        cp.start()
        out_copies.append(cp)
    for cp in out_copies:
        cp.wait()


def make(bq=BQ, bk=BK):
    def f(A_x, A_wqkv, A_wo, B_x, B_wqkv, B_wo, gate_w):
        del B_x
        nq = S // bq
        xt = A_x.reshape(S, D).T
        gw = gate_w.reshape(1, D)
        vm = pl.BlockSpec(memory_space=pltpu.VMEM)
        hbm = pl.BlockSpec(memory_space=pl.ANY)
        out = pl.pallas_call(
            functools.partial(_kernel, bq=bq, bk=bk),
            out_shape=jax.ShapeDtypeStruct((D, S), A_x.dtype),
            in_specs=[hbm] * 5 + [vm],
            out_specs=hbm,
            scratch_shapes=[
                pltpu.VMEM((D, S), jnp.bfloat16),
                pltpu.VMEM((D, 3 * D), jnp.bfloat16),
                pltpu.VMEM((D, 3 * D), jnp.bfloat16),
                pltpu.VMEM((D, D), jnp.bfloat16),
                pltpu.VMEM((D, D), jnp.bfloat16),
                pltpu.VMEM((nq, D, bq), A_x.dtype),
                pltpu.SemaphoreType.DMA((5,)),
                pltpu.SemaphoreType.DMA((nq,)),
                pltpu.VMEM((1968, D), jnp.bfloat16),
                pltpu.VMEM((D, 1024), jnp.bfloat16),
                pltpu.VMEM((8, S, 128), jnp.bfloat16),
                pltpu.VMEM((nq, 2, 464, bq), jnp.bfloat16),
                pltpu.VMEM((2, 512, S), jnp.bfloat16),
                pltpu.VMEM((8, S), jnp.float32),
                pltpu.VMEM((nq, 1024, bq), jnp.bfloat16),
                pltpu.VMEM((S, bq), jnp.float32),
                pltpu.VMEM((S, bq), jnp.float32),
            ],
            compiler_params=pltpu.CompilerParams(vmem_limit_bytes=100 * 2 ** 20),
        )(xt, A_wqkv, B_wqkv, A_wo, B_wo, gw)
        return out.T.reshape(1, S, D)
    return jax.jit(f)


pallas_gated_mix__mha_block__mha_block__prompt_kernel = make()
```

```python
import functools
import os
import numpy as np
import jax
import jax.numpy as jnp
import jax.experimental.pallas as pl
import jax.experimental.pallas.tpu as pltpu

S = 2048
D = 448
H = 16
DH = 28
BQ = 256
BK = 256
TB = 512
LAG = int(os.environ.get('LAG', '1'))
GPI = int(os.environ.get('GPI', '4'))
import contextlib
SC = (lambda n: jax.named_scope(n)) if os.environ.get('SCOPES') else (lambda n: contextlib.nullcontext())
QSCALE = float(DH ** -0.5 * np.log2(np.e))


def _kernel(xt_hbm, wa_hbm, wb_hbm, woa_hbm, wob_hbm, gw_ref, o_hbm,
            xt_s, x_s, w_s, wo_s, o_s, in_sems, x_sems, out_sems,
            wt_s, wot_s, kp_s, qt_s, vt_s, g_s, og_s, ot_s, sA, sB, *, bq, bk, nit=None):
    nq = S // bq
    nch = S // bk
    ntb = S // TB
    f32 = jnp.float32
    bf16 = jnp.bfloat16

    w_cp = [pltpu.make_async_copy(src, w_s.at[m], in_sems.at[m]) for m, src in enumerate((wa_hbm, wb_hbm))]
    wo_cp = [pltpu.make_async_copy(src, wo_s.at[m], in_sems.at[2 + m]) for m, src in enumerate((woa_hbm, wob_hbm))]
    x_cp = [pltpu.make_async_copy(xt_hbm.at[:, pl.ds(i * TB, TB)], xt_s.at[i], x_sems.at[i]) for i in range(ntb)]
    w_cp[0].start()
    x_cp[0].start()

    VOFF = 464
    rowv = jax.lax.broadcasted_iota(jnp.int32, (4, TB), 0)
    vpad = jnp.where(rowv == 0, 1.0, 0.0).astype(f32)
    for m in range(2):
      with SC(f'waitw{m}'):
        w_cp[m].wait()
      with SC(f'proj{m}'):
        if m == 0:
            for c in x_cp[1:]:
                c.start()
            w_cp[1].start()
            for c in wo_cp:
                c.start()
        w_ref = w_s.at[m]
        wt_s[0:D, :] = w_ref[:, 0:512].astype(f32).T[0:D].astype(bf16)
        if m == 0:
            wt_s[D:VOFF, :] = jnp.broadcast_to(gw_ref[...].astype(f32).reshape(1, D), (16, D)).astype(bf16)
        wt_s[VOFF:VOFF + D, :] = w_ref[:, 2 * D:3 * D].astype(f32).T.astype(bf16)
        for i in range(ntb):
            if m == 0:
                x_cp[i].wait()
                x_s[i] = xt_s[i].T
            xtb = xt_s[i]
            xb = x_s[i]
            nrow = VOFF if m == 0 else D
            q = jnp.dot(wt_s[0:nrow, :], xtb, preferred_element_type=f32)
            if m == 0:
                g_s[:, i * TB:(i + 1) * TB] = jax.nn.sigmoid(q[D:D + 8])
            qs = (q[0:D] * QSCALE).astype(bf16)
            for u in range(TB // bq):
                qt_s[i * (TB // bq) + u, m, 0:D, :] = qs[:, u * bq:(u + 1) * bq]
                qt_s[i * (TB // bq) + u, m, D:VOFF, :] = jnp.zeros((16, bq), bf16)
            v = jnp.dot(wt_s[VOFF:VOFF + D, :], xtb, preferred_element_type=f32)
            for h in range(H):
                vh = jnp.concatenate([v[DH * h:DH * h + DH], vpad], axis=0)
                vt_s[m, 32 * h:32 * h + 32, i * TB:(i + 1) * TB] = vh.astype(bf16)
            for g in range(4):
                c0 = D + 112 * g
                k = jnp.dot(xb, w_ref[:, c0:c0 + 128], preferred_element_type=f32)
                kp_s[4 * m + g, i * TB:(i + 1) * TB, :] = k.astype(bf16)

    for m in range(2):
      with SC(f'wot{m}'):
        wo_cp[m].wait()
        wot_s[:, D * m:D * m + D] = wo_s[m].astype(f32).T.astype(bf16)

    row = jax.lax.broadcasted_iota(jnp.int32, (128, bq), 0)

    def qweights(qb, grp, hp):
        m = grp // 4
        g = grp % 4
        w = qt_s[qb, m, pl.ds(pl.multiple_of(g * 112, 16), 128), :]
        lo = hp * DH
        msk = jnp.logical_and(row >= lo, row < lo + DH)
        return jnp.where(msk, w, jnp.zeros_like(w))

    def qk_chunk(w, grp, sb, j, mx):
        kc = kp_s[grp, pl.ds(j * bk, bk), :]
        s = jnp.dot(kc, w, preferred_element_type=f32)
        sb[pl.ds(j * bk, bk), :] = s
        cm = jnp.max(s.reshape(bk // 8, 8, bq), axis=0)
        return cm if mx is None else jnp.maximum(mx, cm)

    def pv_chunk(grp, hp, sb, j, mcur, acc, z):
        s = sb[pl.ds(pl.multiple_of(j * bk + z, 8), bk), :]
        p = jnp.exp2(s - mcur).astype(bf16)
        m = grp // 4
        g = grp % 4
        v = vt_s[m, pl.ds(pl.multiple_of(g * 128 + hp * 32, 32), 32), pl.ds(j * bk, bk)]
        d = jnp.dot(v, p, preferred_element_type=f32)
        return d if acc is None else acc + d

    def step(cur_idx, nxt_idx, mcur, scur, snxt, z):
        mx = None
        acc = None
        if nxt_idx is not None:
            w = qweights(*nxt_idx)
        for j in range(nch + LAG):
            if nxt_idx is not None and j < nch:
                mx = qk_chunk(w, nxt_idx[1], snxt, j, mx)
            if cur_idx is not None and j >= LAG:
                acc = pv_chunk(cur_idx[1], cur_idx[2], scur, j - LAG, mcur, acc, z)
        if cur_idx is not None:
            qb, grp, hp = cur_idx
            gate = g_s[0:1, pl.ds(pl.multiple_of(qb * bq, bq), bq)]
            wgt = jnp.where(grp < 4, gate, 1.0 - gate)
            og_s[DH * hp:DH * hp + DH, :] = acc[0:DH] * (wgt / acc[DH:DH + 1, :])
            if hp == 3:
                ot_s[qb, pl.ds(pl.multiple_of(grp * 112, 16), 112), :] = og_s[...].astype(bf16)
        if nxt_idx is not None:
            return jnp.max(mx, axis=0, keepdims=True)
        return None

    def group(it, mcur, last):
        qb = it // 8
        grp = it % 8
        z = it // 4096
        mcur = step((qb, grp, 0), (qb, grp, 1), mcur, sA, sB, z)
        mcur = step((qb, grp, 1), (qb, grp, 2), mcur, sB, sA, z)
        mcur = step((qb, grp, 2), (qb, grp, 3), mcur, sA, sB, z)
        if last:
            return step((qb, grp, 3), None, mcur, sB, sA, z)
        return step((qb, grp, 3), ((it + 1) // 8, (it + 1) % 8, 0), mcur, sB, sA, z)

    with SC('qk0'):
        m0 = step(None, (0, 0, 0), None, None, sA, 0)
    n_it = nit or nq * 8

    def multi(i, c):
        mc = c[0]
        for u in range(GPI):
            mc = group(i * GPI + u, mc, False)
        return mc, (i + 1) * GPI

    with SC('loop'):
      mlast, it_last = jax.lax.fori_loop(
        0, n_it // GPI - 1, multi, (m0, jnp.int32(0)))
    with SC('lastgroup'):
        for u in range(GPI - 1):
            mlast = group(it_last + u, mlast, False)
        group(it_last + GPI - 1, mlast, True)

    out_copies = []
    OW = 512
    for u in range(S // OW):
      with SC(f'out{u}'):
        rhs = ot_s[u] if bq == OW else jnp.concatenate([ot_s[u * (OW // bq) + v] for v in range(OW // bq)], axis=1)
        ot = jnp.dot(wot_s[...], rhs, preferred_element_type=f32)
        o_s[u] = ot.astype(o_s.dtype)
        cp = pltpu.make_async_copy(o_s.at[u], o_hbm.at[:, pl.ds(u * OW, OW)], out_sems.at[u])
        cp.start()
        out_copies.append(cp)
    with SC('outwait'):
      for cp in out_copies:
        cp.wait()


def make(bq=BQ, bk=BK, nit=None):
    def f(A_x, A_wqkv, A_wo, B_x, B_wqkv, B_wo, gate_w):
        del B_x
        nq = S // bq
        bf16 = jnp.bfloat16
        xt = A_x.reshape(S, D).T
        vm = pl.BlockSpec(memory_space=pltpu.VMEM)
        hbm = pl.BlockSpec(memory_space=pl.ANY)
        out = pl.pallas_call(
            functools.partial(_kernel, bq=bq, bk=bk, nit=nit),
            out_shape=jax.ShapeDtypeStruct((D, S), A_x.dtype),
            in_specs=[hbm] * 5 + [vm],
            out_specs=hbm,
            scratch_shapes=[
                pltpu.VMEM((S // TB, D, TB), bf16),
                pltpu.VMEM((S // TB, TB, D), bf16),
                pltpu.VMEM((2, D, 3 * D), bf16),
                pltpu.VMEM((2, D, D), bf16),
                pltpu.VMEM((S // 512, D, 512), A_x.dtype),
                pltpu.SemaphoreType.DMA((4,)),
                pltpu.SemaphoreType.DMA((S // TB,)),
                pltpu.SemaphoreType.DMA((S // 512,)),
                pltpu.VMEM((2 * D + 16, D), bf16),
                pltpu.VMEM((D, 2 * D), bf16),
                pltpu.VMEM((8, S, 128), bf16),
                pltpu.VMEM((nq, 2, 464, bq), bf16),
                pltpu.VMEM((2, 512, S), bf16),
                pltpu.VMEM((8, S), jnp.float32),
                pltpu.VMEM((112, bq), jnp.float32),
                pltpu.VMEM((nq, 2 * D, bq), bf16),
                pltpu.VMEM((S, bq), jnp.float32),
                pltpu.VMEM((S, bq), jnp.float32),
            ],
            compiler_params=pltpu.CompilerParams(vmem_limit_bytes=100 * 2 ** 20),
        )(xt, A_wqkv, B_wqkv, A_wo, B_wo, gate_w)
        return out.T.reshape(1, S, D)
    return jax.jit(f)


pallas_gated_mix__mha_block__mha_block__prompt_kernel = make()
```

```python
import functools
import numpy as np
import jax
import jax.numpy as jnp
import jax.experimental.pallas as pl
import jax.experimental.pallas.tpu as pltpu

S = 2048
D = 448
H = 16
DH = 28
BQ = 256
BK = 256
TB = 512
LAG = 1
GPI = 4
QSCALE = float(DH ** -0.5 * np.log2(np.e))


def _kernel(xt_hbm, wa_hbm, wb_hbm, woa_hbm, wob_hbm, gw_ref, o_hbm,
            xt_s, w_s, wo_s, o_s, in_sems, x_sems, out_sems,
            wt_s, wot_s, kp_s, qt_s, vt_s, g_s, og_s, ot_s, sA, sB, *, bq, bk, nit=None):
    nq = S // bq
    nch = S // bk
    ntb = S // TB
    f32 = jnp.float32
    bf16 = jnp.bfloat16

    WSPLIT = ((0, 512), (2 * D, 3 * D), (512, 2 * D))
    wa_cp = [pltpu.make_async_copy(wa_hbm.at[:, lo:hi], w_s.at[0, :, lo:hi], in_sems.at[j])
             for j, (lo, hi) in enumerate(WSPLIT)]
    wb_cp = pltpu.make_async_copy(wb_hbm, w_s.at[1], in_sems.at[3])
    wo_cp = [pltpu.make_async_copy(src, wo_s.at[m], in_sems.at[4 + m]) for m, src in enumerate((woa_hbm, wob_hbm))]
    x_cp = [pltpu.make_async_copy(xt_hbm.at[:, pl.ds(i * TB, TB)], xt_s.at[i], x_sems.at[i]) for i in range(ntb)]
    wa_cp[0].start()
    x_cp[0].start()

    KOFF = 464
    VOFF = 912
    rowv = jax.lax.broadcasted_iota(jnp.int32, (4, TB), 0)
    vpad = jnp.where(rowv == 0, 1.0, 0.0).astype(f32)

    def prep_wq(m):
        wt_s[m, 0:D, :] = w_s[m, :, 0:512].astype(f32).T[0:D].astype(bf16)
        if m == 0:
            wt_s[m, D:KOFF, :] = jnp.broadcast_to(gw_ref[...].astype(f32).reshape(1, D), (16, D)).astype(bf16)

    def prep_wk(m):
        wt_s[m, KOFF:VOFF, :] = w_s[m, :, 384:2 * D].astype(f32).T[64:].astype(bf16)

    def prep_wv(m):
        wt_s[m, VOFF:VOFF + D, :] = w_s[m, :, 2 * D:3 * D].astype(f32).T.astype(bf16)

    def prep_wot(m):
        wo_cp[m].wait()
        wot_s[:, D * m:D * m + D] = wo_s[m].astype(f32).T.astype(bf16)

    def proj_k(m, i):
        kt = jnp.dot(wt_s[m, KOFF:VOFF, :], xt_s[i], preferred_element_type=f32)
        for g in range(4):
            kw = jnp.concatenate([kt[112 * g:112 * g + 112], jnp.zeros((16, TB), f32)], axis=0)
            kp_s[4 * m + g, i * TB:(i + 1) * TB, :] = kw.T.astype(bf16)

    def proj_q(m, i):
        nrow = KOFF if m == 0 else D
        q = jnp.dot(wt_s[m, 0:nrow, :], xt_s[i], preferred_element_type=f32)
        if m == 0:
            g_s[:, i * TB:(i + 1) * TB] = jax.nn.sigmoid(q[D:D + 8])
        qs = (q[0:D] * QSCALE).astype(bf16)
        for u in range(TB // bq):
            qt_s[i * (TB // bq) + u, m, 0:D, :] = qs[:, u * bq:(u + 1) * bq]
            qt_s[i * (TB // bq) + u, m, D:KOFF, :] = jnp.zeros((16, bq), bf16)

    def proj_v(m, i):
        v = jnp.dot(wt_s[m, VOFF:VOFF + D, :], xt_s[i], preferred_element_type=f32)
        for h in range(H):
            vh = jnp.concatenate([v[DH * h:DH * h + DH], vpad], axis=0)
            vt_s[m, 32 * h:32 * h + 32, i * TB:(i + 1) * TB] = vh.astype(bf16)

    wa_cp[0].wait()
    x_cp[0].wait()
    wa_cp[1].start()
    wa_cp[2].start()
    prep_wq(0)
    proj_q(0, 0)
    wa_cp[1].wait()
    wa_cp[2].wait()
    x_cp[1].start()
    x_cp[2].start()
    prep_wv(0)
    prep_wk(0)
    proj_v(0, 0)
    proj_k(0, 0)
    for i in range(1, ntb):
        x_cp[i].wait()
        if i == 1:
            x_cp[3].start()
            wb_cp.start()
        if i == 2:
            wb_cp.wait()
            for c in wo_cp:
                c.start()
        proj_q(0, i)
        if i == 2:
            prep_wq(1)
        proj_v(0, i)
        if i == 3:
            prep_wv(1)
        proj_k(0, i)
        if i == 3:
            prep_wk(1)
    for i in range(ntb):
        proj_q(1, i)
        proj_v(1, i)
        proj_k(1, i)

    row = jax.lax.broadcasted_iota(jnp.int32, (128, bq), 0)

    def qweights(qb, grp, hp):
        m = grp // 4
        g = grp % 4
        w = qt_s[qb, m, pl.ds(pl.multiple_of(g * 112, 16), 128), :]
        lo = hp * DH
        msk = jnp.logical_and(row >= lo, row < lo + DH)
        return jnp.where(msk, w, jnp.zeros_like(w))

    def qk_chunk(w, grp, sb, j, mx):
        kc = kp_s[grp, pl.ds(j * bk, bk), :]
        s = jnp.dot(kc, w, preferred_element_type=f32)
        sb[pl.ds(j * bk, bk), :] = s
        cm = jnp.max(s.reshape(bk // 8, 8, bq), axis=0)
        return cm if mx is None else jnp.maximum(mx, cm)

    def pv_chunk(grp, hp, sb, j, mcur, acc, z):
        s = sb[pl.ds(pl.multiple_of(j * bk + z, 8), bk), :]
        p = jnp.exp2(s - mcur).astype(bf16)
        m = grp // 4
        g = grp % 4
        v = vt_s[m, pl.ds(pl.multiple_of(g * 128 + hp * 32, 32), 32), pl.ds(j * bk, bk)]
        d = jnp.dot(v, p, preferred_element_type=f32)
        return d if acc is None else acc + d

    def step(cur_idx, nxt_idx, mcur, scur, snxt, z):
        mx = None
        acc = None
        if nxt_idx is not None:
            w = qweights(*nxt_idx)
        for j in range(nch + LAG):
            if nxt_idx is not None and j < nch:
                mx = qk_chunk(w, nxt_idx[1], snxt, j, mx)
            if cur_idx is not None and j >= LAG:
                acc = pv_chunk(cur_idx[1], cur_idx[2], scur, j - LAG, mcur, acc, z)
        if cur_idx is not None:
            qb, grp, hp = cur_idx
            gate = g_s[0:1, pl.ds(pl.multiple_of(qb * bq, bq), bq)]
            wgt = jnp.where(grp < 4, gate, 1.0 - gate)
            og_s[DH * hp:DH * hp + DH, :] = acc[0:DH] * (wgt / acc[DH:DH + 1, :])
            if hp == 3:
                ot_s[qb, pl.ds(pl.multiple_of(grp * 112, 16), 112), :] = og_s[...].astype(bf16)
        if nxt_idx is not None:
            return jnp.max(mx, axis=0, keepdims=True)
        return None

    def group(it, mcur, last):
        qb = it // 8
        grp = it % 8
        z = it // 4096
        mcur = step((qb, grp, 0), (qb, grp, 1), mcur, sA, sB, z)
        mcur = step((qb, grp, 1), (qb, grp, 2), mcur, sB, sA, z)
        mcur = step((qb, grp, 2), (qb, grp, 3), mcur, sA, sB, z)
        if last:
            return step((qb, grp, 3), None, mcur, sB, sA, z)
        return step((qb, grp, 3), ((it + 1) // 8, (it + 1) % 8, 0), mcur, sB, sA, z)

    m0 = step(None, (0, 0, 0), None, None, sA, 0)
    n_it = nit or nq * 8

    def multi(i, c):
        mc = c[0]
        for u in range(GPI):
            mc = group(i * GPI + u, mc, False)
        return mc, (i + 1) * GPI

    mlast, it_last = jax.lax.fori_loop(
        0, n_it // GPI - 1, multi, (m0, jnp.int32(0)))
    for u in range(GPI - 1):
        mlast = group(it_last + u, mlast, False)
        if u < 2:
            prep_wot(u)
    group(it_last + GPI - 1, mlast, True)

    out_copies = []
    OW = 512
    for u in range(S // OW):
        rhs = ot_s[u] if bq == OW else jnp.concatenate([ot_s[u * (OW // bq) + v] for v in range(OW // bq)], axis=1)
        ot = jnp.dot(wot_s[...], rhs, preferred_element_type=f32)
        o_s[u] = ot.astype(o_s.dtype)
        cp = pltpu.make_async_copy(o_s.at[u], o_hbm.at[:, pl.ds(u * OW, OW)], out_sems.at[u])
        cp.start()
        out_copies.append(cp)
    for cp in out_copies:
        cp.wait()


def make(bq=BQ, bk=BK, nit=None):
    def f(A_x, A_wqkv, A_wo, B_x, B_wqkv, B_wo, gate_w):
        del B_x
        nq = S // bq
        bf16 = jnp.bfloat16
        xt = A_x.reshape(S, D).T
        vm = pl.BlockSpec(memory_space=pltpu.VMEM)
        hbm = pl.BlockSpec(memory_space=pl.ANY)
        out = pl.pallas_call(
            functools.partial(_kernel, bq=bq, bk=bk, nit=nit),
            out_shape=jax.ShapeDtypeStruct((D, S), A_x.dtype),
            in_specs=[hbm] * 5 + [vm],
            out_specs=hbm,
            scratch_shapes=[
                pltpu.VMEM((S // TB, D, TB), bf16),
                pltpu.VMEM((2, D, 3 * D), bf16),
                pltpu.VMEM((2, D, D), bf16),
                pltpu.VMEM((S // 512, D, 512), A_x.dtype),
                pltpu.SemaphoreType.DMA((6,)),
                pltpu.SemaphoreType.DMA((S // TB,)),
                pltpu.SemaphoreType.DMA((S // 512,)),
                pltpu.VMEM((2, 3 * D + 16, D), bf16),
                pltpu.VMEM((D, 2 * D), bf16),
                pltpu.VMEM((8, S, 128), bf16),
                pltpu.VMEM((nq, 2, 464, bq), bf16),
                pltpu.VMEM((2, 512, S), bf16),
                pltpu.VMEM((8, S), jnp.float32),
                pltpu.VMEM((112, bq), jnp.float32),
                pltpu.VMEM((nq, 2 * D, bq), bf16),
                pltpu.VMEM((S, bq), jnp.float32),
                pltpu.VMEM((S, bq), jnp.float32),
            ],
            compiler_params=pltpu.CompilerParams(vmem_limit_bytes=100 * 2 ** 20),
        )(xt, A_wqkv, B_wqkv, A_wo, B_wo, gate_w)
        return out.T.reshape(1, S, D)
    return jax.jit(f)


pallas_gated_mix__mha_block__mha_block__prompt_kernel = make()
```

```python
import functools
import numpy as np
import jax
import jax.numpy as jnp
import jax.experimental.pallas as pl
import jax.experimental.pallas.tpu as pltpu

S = 2048
D = 448
H = 16
DH = 28
BQ = 256
BK = 256
TB = 512
LAG = 1
GPI = 4
QSCALE = float(DH ** -0.5 * np.log2(np.e))


def _kernel(xt_hbm, wa_hbm, wb_hbm, woa_hbm, wob_hbm, gw_ref, o_hbm,
            xt_s, w_s, wo_s, o_s, in_sems, x_sems, out_sems,
            wt_s, wot_s, kp_s, qt_s, vt_s, g_s, og_s, ot_s, sA, sB, *, bq, bk, nit=None):
    nq = S // bq
    nch = S // bk
    ntb = S // TB
    f32 = jnp.float32
    bf16 = jnp.bfloat16

    WSPLIT = ((0, 512), (2 * D, 3 * D), (512, 2 * D))
    wa_cp = [pltpu.make_async_copy(wa_hbm.at[:, lo:hi], w_s.at[0, :, lo:hi], in_sems.at[j])
             for j, (lo, hi) in enumerate(WSPLIT)]
    wb_cp = pltpu.make_async_copy(wb_hbm, w_s.at[1], in_sems.at[3])
    wo_cp = [pltpu.make_async_copy(src, wo_s.at[m], in_sems.at[4 + m]) for m, src in enumerate((woa_hbm, wob_hbm))]
    x_cp = [pltpu.make_async_copy(xt_hbm.at[:, pl.ds(i * TB, TB)], xt_s.at[i], x_sems.at[i]) for i in range(ntb)]
    wa_cp[0].start()
    x_cp[0].start()

    KOFF = 464
    VOFF = 912
    rowv = jax.lax.broadcasted_iota(jnp.int32, (4, TB), 0)
    vpad = jnp.where(rowv == 0, 1.0, 0.0).astype(f32)

    def prep_wq(m):
        wt_s[m, 0:D, :] = w_s[m, :, 0:512].astype(f32).T[0:D].astype(bf16)
        if m == 0:
            wt_s[m, D:KOFF, :] = jnp.broadcast_to(gw_ref[...].astype(f32).reshape(1, D), (16, D)).astype(bf16)

    def prep_wk(m):
        wt_s[m, KOFF:VOFF, :] = w_s[m, :, 384:2 * D].astype(f32).T[64:].astype(bf16)

    def prep_wv(m):
        wt_s[m, VOFF:VOFF + D, :] = w_s[m, :, 2 * D:3 * D].astype(f32).T.astype(bf16)

    def prep_wot(m):
        wo_cp[m].wait()
        wot_s[:, D * m:D * m + D] = wo_s[m].astype(f32).T.astype(bf16)

    def proj_k(m, i):
        kt = jnp.dot(wt_s[m, KOFF:VOFF, :], xt_s[i], preferred_element_type=f32)
        for g in range(4):
            kw = jnp.concatenate([kt[112 * g:112 * g + 112], jnp.zeros((16, TB), f32)], axis=0)
            kp_s[4 * m + g, i * TB:(i + 1) * TB, :] = kw.T.astype(bf16)

    def proj_q(m, i):
        nrow = KOFF if m == 0 else D
        q = jnp.dot(wt_s[m, 0:nrow, :], xt_s[i], preferred_element_type=f32)
        if m == 0:
            g_s[:, i * TB:(i + 1) * TB] = jax.nn.sigmoid(q[D:D + 8])
        qs = (q[0:D] * QSCALE).astype(bf16)
        for u in range(TB // bq):
            qt_s[i * (TB // bq) + u, m, 0:D, :] = qs[:, u * bq:(u + 1) * bq]
            qt_s[i * (TB // bq) + u, m, D:KOFF, :] = jnp.zeros((16, bq), bf16)

    def proj_v(m, i):
        v = jnp.dot(wt_s[m, VOFF:VOFF + D, :], xt_s[i], preferred_element_type=f32)
        for h in range(H):
            vh = jnp.concatenate([v[DH * h:DH * h + DH], vpad], axis=0)
            vt_s[m, 32 * h:32 * h + 32, i * TB:(i + 1) * TB] = vh.astype(bf16)

    wa_cp[0].wait()
    wa_cp[1].start()
    wa_cp[2].start()
    prep_wq(0)
    x_cp[0].wait()
    proj_q(0, 0)
    wa_cp[1].wait()
    wa_cp[2].wait()
    x_cp[1].start()
    x_cp[2].start()
    prep_wv(0)
    prep_wk(0)
    proj_v(0, 0)
    proj_k(0, 0)
    x_cp[1].wait()
    x_cp[3].start()
    wb_cp.start()
    for i in range(1, ntb):
        proj_q(0, i)
        if i == 2:
            prep_wq(1)
        proj_v(0, i)
        if i == 3:
            prep_wv(1)
        if i < 3:
            x_cp[i + 1].wait()
        if i == 1:
            wb_cp.wait()
            for c in wo_cp:
                c.start()
        proj_k(0, i)
        if i == 3:
            prep_wk(1)
    for i in range(ntb):
        proj_q(1, i)
        proj_v(1, i)
        proj_k(1, i)

    row = jax.lax.broadcasted_iota(jnp.int32, (128, bq), 0)

    def qweights(qb, grp, hp):
        m = grp // 4
        g = grp % 4
        w = qt_s[qb, m, pl.ds(pl.multiple_of(g * 112, 16), 128), :]
        lo = hp * DH
        msk = jnp.logical_and(row >= lo, row < lo + DH)
        return jnp.where(msk, w, jnp.zeros_like(w))

    def qk_chunk(w, grp, sb, j, mx):
        kc = kp_s[grp, pl.ds(j * bk, bk), :]
        s = jnp.dot(kc, w, preferred_element_type=f32)
        sb[pl.ds(j * bk, bk), :] = s
        cm = jnp.max(s.reshape(bk // 8, 8, bq), axis=0)
        return cm if mx is None else jnp.maximum(mx, cm)

    def pv_chunk(grp, hp, sb, j, mcur, acc, z):
        s = sb[pl.ds(pl.multiple_of(j * bk + z, 8), bk), :]
        p = jnp.exp2(s - mcur).astype(bf16)
        m = grp // 4
        g = grp % 4
        v = vt_s[m, pl.ds(pl.multiple_of(g * 128 + hp * 32, 32), 32), pl.ds(j * bk, bk)]
        d = jnp.dot(v, p, preferred_element_type=f32)
        return d if acc is None else acc + d

    def step(cur_idx, nxt_idx, mcur, scur, snxt, z):
        mx = None
        acc = None
        if nxt_idx is not None:
            w = qweights(*nxt_idx)
        for j in range(nch + LAG):
            if nxt_idx is not None and j < nch:
                mx = qk_chunk(w, nxt_idx[1], snxt, j, mx)
            if cur_idx is not None and j >= LAG:
                acc = pv_chunk(cur_idx[1], cur_idx[2], scur, j - LAG, mcur, acc, z)
        if cur_idx is not None:
            qb, grp, hp = cur_idx
            gate = g_s[0:1, pl.ds(pl.multiple_of(qb * bq, bq), bq)]
            wgt = jnp.where(grp < 4, gate, 1.0 - gate)
            og_s[DH * hp:DH * hp + DH, :] = acc[0:DH] * (wgt / acc[DH:DH + 1, :])
            if hp == 3:
                ot_s[qb, pl.ds(pl.multiple_of(grp * 112, 16), 112), :] = og_s[...].astype(bf16)
        if nxt_idx is not None:
            return jnp.max(mx, axis=0, keepdims=True)
        return None

    def group(it, mcur, last):
        qb = it // 8
        grp = it % 8
        z = it // 4096
        mcur = step((qb, grp, 0), (qb, grp, 1), mcur, sA, sB, z)
        mcur = step((qb, grp, 1), (qb, grp, 2), mcur, sB, sA, z)
        mcur = step((qb, grp, 2), (qb, grp, 3), mcur, sA, sB, z)
        if last:
            return step((qb, grp, 3), None, mcur, sB, sA, z)
        return step((qb, grp, 3), ((it + 1) // 8, (it + 1) % 8, 0), mcur, sB, sA, z)

    m0 = step(None, (0, 0, 0), None, None, sA, 0)
    n_it = nit or nq * 8

    def multi(i, c):
        mc = c[0]
        for u in range(GPI):
            mc = group(i * GPI + u, mc, False)
        return mc, (i + 1) * GPI

    mlast, it_last = jax.lax.fori_loop(
        0, n_it // GPI - 1, multi, (m0, jnp.int32(0)))
    for u in range(GPI - 1):
        mlast = group(it_last + u, mlast, False)
        if u < 2:
            prep_wot(u)
    group(it_last + GPI - 1, mlast, True)

    out_copies = []
    OW = 512
    for u in range(S // OW):
        rhs = ot_s[u] if bq == OW else jnp.concatenate([ot_s[u * (OW // bq) + v] for v in range(OW // bq)], axis=1)
        ot = jnp.dot(wot_s[...], rhs, preferred_element_type=f32)
        o_s[u] = ot.astype(o_s.dtype)
        cp = pltpu.make_async_copy(o_s.at[u], o_hbm.at[:, pl.ds(u * OW, OW)], out_sems.at[u])
        cp.start()
        out_copies.append(cp)
    for cp in out_copies:
        cp.wait()


def make(bq=BQ, bk=BK, nit=None):
    def f(A_x, A_wqkv, A_wo, B_x, B_wqkv, B_wo, gate_w):
        del B_x
        nq = S // bq
        bf16 = jnp.bfloat16
        xt = A_x.reshape(S, D).T
        vm = pl.BlockSpec(memory_space=pltpu.VMEM)
        hbm = pl.BlockSpec(memory_space=pl.ANY)
        out = pl.pallas_call(
            functools.partial(_kernel, bq=bq, bk=bk, nit=nit),
            out_shape=jax.ShapeDtypeStruct((D, S), A_x.dtype),
            in_specs=[hbm] * 5 + [vm],
            out_specs=hbm,
            scratch_shapes=[
                pltpu.VMEM((S // TB, D, TB), bf16),
                pltpu.VMEM((2, D, 3 * D), bf16),
                pltpu.VMEM((2, D, D), bf16),
                pltpu.VMEM((S // 512, D, 512), A_x.dtype),
                pltpu.SemaphoreType.DMA((6,)),
                pltpu.SemaphoreType.DMA((S // TB,)),
                pltpu.SemaphoreType.DMA((S // 512,)),
                pltpu.VMEM((2, 3 * D + 16, D), bf16),
                pltpu.VMEM((D, 2 * D), bf16),
                pltpu.VMEM((8, S, 128), bf16),
                pltpu.VMEM((nq, 2, 464, bq), bf16),
                pltpu.VMEM((2, 512, S), bf16),
                pltpu.VMEM((8, S), jnp.float32),
                pltpu.VMEM((112, bq), jnp.float32),
                pltpu.VMEM((nq, 2 * D, bq), bf16),
                pltpu.VMEM((S, bq), jnp.float32),
                pltpu.VMEM((S, bq), jnp.float32),
            ],
            compiler_params=pltpu.CompilerParams(vmem_limit_bytes=100 * 2 ** 20),
        )(xt, A_wqkv, B_wqkv, A_wo, B_wo, gate_w)
        return out.T.reshape(1, S, D)
    return jax.jit(f)


pallas_gated_mix__mha_block__mha_block__prompt_kernel = make()
```
